```python
import jax
import jax.numpy as jnp

def _softmax(x, axis=-1):
    return jax.nn.softmax(x, axis=axis)
def _gelu(x):
    return jax.nn.gelu(x, approximate=True)
def _silu(x):
    return jax.nn.silu(x)
def _sigmoid(x):
    return jax.nn.sigmoid(x)
def _layernorm(x, axis=-1, eps=1e-5):
    m = jnp.mean(x, axis=axis, keepdims=True)
    v = jnp.var(x, axis=axis, keepdims=True)
    return (x - m) / jnp.sqrt(v + eps)
def _scatter_add(tgt, idx, src, axis=0):
    return tgt.at[idx].add(src)
def _segment_sum(src, seg, n):
    return jax.ops.segment_sum(src, seg, n)
class _Rng:
    def __init__(self, key):
        self._k = key
    def _next(self):
        self._k, sub = jax.random.split(self._k)
        return sub
    def normal(self, shape):
        return jax.random.normal(self._next(), shape, dtype=jnp.bfloat16)
    def randint(self, lo, hi, shape):
        return jax.random.randint(self._next(), shape, lo, hi, dtype=jnp.int32)
    def uniform(self, shape, lo=0.0, hi=1.0):
        return jax.random.uniform(self._next(), shape, jnp.bfloat16, lo, hi)
    def permutation(self, n):
        return jax.random.permutation(self._next(), n)


kernel_name = 'standalone__batchnorm__prompt'

def setup_inputs():
    _rng = _Rng(jax.random.key(int.from_bytes(__import__("os").urandom(4), "little")))
    _w = (lambda a: (lambda t: t.astype(jnp.bfloat16) if jnp.issubdtype(t.dtype, jnp.floating) else t)(jnp.asarray(a)))
    B, S, C = 2, 2048, 1024
    K = 3
    return {
        "x": _w((lambda *s: _rng.normal(s) * 0.05)(B, S, C)),
        "w": _w((lambda *s: _rng.normal(s) * 0.05)(K, C, C) * (1.0 / (K * C) ** 0.5)),
        "mean": _w((lambda *s: _rng.normal(s) * 0.05)(C) * 0.1),
        "var": _w(jnp.abs((lambda *s: _rng.normal(s) * 0.05)(C)) + 0.5),
        "g": _w((lambda *s: _rng.normal(s) * 0.05)(C) + 1.0),
        "b": _w((lambda *s: _rng.normal(s) * 0.05)(C) * 0.1),
    }

def reference(x, w, mean, var, g, b):
    K = 3
    P = K // 2
    S = x.shape[1]
    xp = jnp.pad(x, ((0, 0), (P, P), (0, 0)))
    y = sum(jnp.einsum('bsc,cd->bsd', xp[:, k:k + S, :], w[k]) for k in range(K))
    inv_std = 1.0 / jnp.sqrt(var + 1e-5)
    y = (y - mean) * (g * inv_std) + b
    return _silu(y)
```

```python
import functools

import jax
import jax.numpy as jnp
import jax.experimental.pallas as pl
import jax.experimental.pallas.tpu as pltpu

F32, BF16, U32 = jnp.float32, jnp.bfloat16, jnp.uint32

B, S, C = 2, 2048, 1024
NC = C // 128
T = 128
NM = S // 4 // T
NI = B * NM
NA = 2
HALO = 16

P, Q = 0.625, 1.5
P2, Q2 = P * P, Q * Q
F0, FP, FQ = P2 * Q2, 2 * P2 * (P2 - Q2), 2 * Q2 * (Q2 - P2)

UNITS_A = [(0, 0), (0, 1), (1, 0), (1, 1)] + [(it, n) for n in range(2, NC) for it in range(NA)]
WAITS = {1: ['W1'], 2: ['X1'], 3: ['W2'], 5: ['W3', 'W4'], 9: ['W5', 'W6', 'W7'], 11: ['X2']}
PRE = {1: ['U1'], 2: ['V1']}
U_SIDE = {2 * n - 1: n for n in range(2, NC)}
V_SIDE = {11: [0, 1], 12: [2, 3, 4], 13: [5], 14: [6, 7]}
STARTS = {'pro': ['W0', 'X0', 'W1'], 'w0': ['X1'], 0: ['W2'], 1: ['W3'], 2: ['W4', 'W5'], 3: ['W6'],
          4: ['W7'], 5: ['X2'], 7: ['X3'], 9: ['X4'], 11: ['X5'], 13: ['X6'], 15: ['X7']}
SLOT_OFFSET = 10
V_UNITS = 5


def _interleave(lists):
    tagged = []
    for tasks in lists:
        for j, t in enumerate(tasks):
            tagged.append(((j + 0.5) / len(tasks), t))
    tagged.sort(key=lambda a: a[0])
    return [t for _, t in tagged]


def _kernel(x_hbm, w_hbm, mean_hbm, var_hbm, g_hbm, b_hbm, o_hbm,
            xs, wr, us, vs, ms, os_, mean_v, var_v, g_v, b_v, xsem, wsem, osem, psem):
    xu, ou, wru = xs.bitcast(U32), os_.bitcast(U32), wr.bitcast(U32)
    as_bf16 = lambda v: pltpu.bitcast(v, BF16)
    lo = lambda u: pltpu.unpack_elementwise(u, index=0, packed_dtype=BF16, unpacked_dtype=F32)
    hi = lambda u: pltpu.unpack_elementwise(u, index=1, packed_dtype=BF16, unpacked_dtype=F32)
    pack = lambda a, b: pltpu.pack_elementwise([a, b], packed_dtype=BF16)

    def x_copies(b, m, it):
        r0 = 0 if m == 0 else m * 4 * T + HALO
        r1 = min((m + 1) * 4 * T + HALO, S)
        return [pltpu.make_async_copy(
            x_hbm.at[b, pl.ds(r0, r1 - r0), pl.ds(c * 128, 128)],
            xs.at[b, c, pl.ds(HALO + r0, r1 - r0), :], xsem.at[it]) for c in range(NC)]

    def w_copies(n):
        return [pltpu.make_async_copy(
            w_hbm.at[k, :, pl.ds(n * 128, 128)], wr.at[k, n], wsem.at[n]) for k in range(3)]

    def o_copy(it, n):
        b = it // NM
        m = it - b * NM
        return pltpu.make_async_copy(
            os_.at[it, n], o_hbm.at[b, pl.ds(m * 4 * T, 4 * T), pl.ds(n * 128, 128)], osem.at[0])

    def group(name):
        k = int(name[1:])
        return x_copies(k // NM, k % NM, k) if name[0] == 'X' else w_copies(k)

    def start(key):
        for name in STARTS.get(key, []):
            for cp in group(name):
                cp.start(priority=0 if name == 'W0' else 1)

    def wait(name):
        for cp in group(name):
            cp.wait()

    start('pro')
    small = [pltpu.make_async_copy(src, dst, psem.at[0]) for src, dst in
             zip((mean_hbm, var_hbm, g_hbm, b_hbm), (mean_v, var_v, g_v, b_v))]
    for cp in small:
        cp.start()
    zero8 = jnp.zeros((8, 128), U32)
    for b in range(B):
        for c in range(NC):
            xu[b, c, pl.ds(0, 8), :] = zero8
            xu[b, c, pl.ds((HALO + S) // 2, 8), :] = zero8
    for cp in small:
        cp.wait()

    mean, var, g, beta = (r[...].astype(F32).reshape(1, C) for r in (mean_v, var_v, g_v, b_v))
    scale = g * (1.0 / jnp.sqrt(var + 1e-5))
    shift = beta - mean * scale
    scale, shift = 0.5 * scale, 0.5 * shift
    zero = jnp.where(pltpu.bitcast(jnp.broadcast_to(var[:, 0:128] * 0.0, (8, 128)), U32) == 12345,
                     jnp.uint32(1), jnp.uint32(0))

    def v_chunk(b, m, slot, c, j):
        if isinstance(m, int):
            xv = xu.at[b, c]
            base = HALO // 2 + m * 2 * T + j * 32
        else:
            xv = xu.at[b, c, pl.ds(pl.multiple_of(m * 2 * T, 8), 2 * T + HALO), :]
            base = HALO // 2 + j * 32
        res = []
        for par in range(2):
            o = base + 2 * par
            prev, cur, nxt, last = (xv[pl.ds(o + k, 8, stride=4), :] for k in (-1, 0, 1, 2))
            d0, d1, d2, d3, d4, d5 = hi(prev), lo(cur), hi(cur), lo(nxt), hi(nxt), lo(last)
            eq = d4 - Q2 * d2
            oq = d3 - Q2 * d1
            ep = d4 - P2 * d2
            op = d3 - P2 * d1
            v0 = ep - Q2 * (d2 - P2 * d0)
            v5 = (d5 - P2 * d3) - Q2 * op
            poq = P * oq
            qop = Q * op
            res.append((v0, eq + poq, eq - poq, ep + qop, ep - qop, v5))
        for i in range(6):
            r = pack(res[0][i], res[1][i])
            vs[slot, i, c, pl.ds(j * 8, 8), :] = r
        return r

    def u_chunk(n, j):
        w = [wru[k, n, pl.ds(j * 8, 8), :] for k in range(3)]
        res = []
        for half in (lo, hi):
            w0, w1, w2 = half(w[0]), half(w[1]), half(w[2])
            e, o = w0 + P2 * w2, P * w1
            e2, o2 = w0 + Q2 * w2, Q * w1
            res.append((e + o, e - o, e2 + o2, e2 - o2))
        for i in range(4):
            r = pack(res[0][i], res[1][i])
            us[i, n, pl.ds(j * 8, 8), :] = r
        return r

    def out_chunk(it, n, mslot, j):
        m0, m1, m2, m3, m4, m5 = (ms[mslot, i, pl.ds(j * 8, 8), :] for i in range(6))
        a = scale[:, n * 128:(n + 1) * 128]
        c0 = shift[:, n * 128:(n + 1) * 128]
        sp, tp = m1 + m2, m1 - m2
        sq, tq = m3 + m4, m3 - m4
        h0 = m0 * (a * (1 / F0)) + sp * (a * (1 / FP)) + sq * (a * (1 / FQ)) + c0
        h1 = tp * (a * (P / FP)) + tq * (a * (Q / FQ)) + c0
        h2 = sp * (a * (P2 / FP)) + sq * (a * (Q2 / FQ)) + c0
        h3 = tp * (a * (P2 * P / FP)) + tq * (a * (Q2 * Q / FQ)) + m5 * a + c0
        y0, y1, y2, y3 = (h + h * jnp.tanh(h) for h in (h0, h1, h2, h3))
        ov = ou.at[it, n]
        ov[pl.ds(16 * j, 8, stride=2), :] = pack(y0, y1)
        r = pack(y2, y3)
        ov[pl.ds(16 * j + 1, 8, stride=2), :] = r
        return r

    def weights(i, n):
        src = (wru.at[0], us.at[0], us.at[1], us.at[2], us.at[3], wru.at[2])[i]
        return as_bf16(src[n])

    def run_unit(slot, n, mslot, side):
        rc = T // 16
        nslots = 6 * 2 * rc
        tied = {}
        for j, t in enumerate(side):
            s = SLOT_OFFSET + int(j * (nslots - SLOT_OFFSET) / len(side))
            tied.setdefault(min(nslots - 1, s), []).append(t)
        for i in range(6):
            dep = {}
            for h in range(2):
                for r in range(rc):
                    for t in tied.get((i * 2 + h) * rc + r, []):
                        d = t() & zero
                        key = (h * (NC // 2), r)
                        dep[key] = d if key not in dep else (dep[key] | d)
            parts = []
            for c in range(NC):
                full = vs[slot, i, c]
                if any(cc == c for cc, _ in dep):
                    full = jnp.concatenate(
                        [(full[8 * r:8 * r + 8] | dep[(c, r)]) if (c, r) in dep else full[8 * r:8 * r + 8]
                         for r in range(rc)], axis=0)
                parts.append(as_bf16(full))
            ms[mslot, i] = jnp.dot(jnp.concatenate(parts, axis=1), weights(i, n),
                                   preferred_element_type=F32)

    v_slot = lambda it: it + 2 if it < NA else it % 2

    wait('W0')
    start('w0')
    for j in range(C // 16):
        u_chunk(0, j)
    wait('X0')
    for c in range(NC):
        for j in range(T // 16):
            v_chunk(0, 0, v_slot(0), c, j)

    for u, (it, n) in enumerate(UNITS_A):
        for name in WAITS.get(u, []):
            wait(name)
        start(u)
        for name in PRE.get(u, []):
            k = int(name[1:])
            if name[0] == 'U':
                for j in range(C // 16):
                    u_chunk(k, j)
            else:
                for c in range(NC):
                    for j in range(T // 16):
                        v_chunk(k // NM, k % NM, v_slot(k), c, j)
        side = []
        if u in U_SIDE:
            side.append([functools.partial(u_chunk, U_SIDE[u], j) for j in range(C // 16)])
        if u in V_SIDE:
            side.append([functools.partial(v_chunk, NA // NM, NA % NM, v_slot(NA), c, j)
                         for c in V_SIDE[u] for j in range(T // 16)])
        if u > 0:
            pit, pn = UNITS_A[u - 1]
            side.append([functools.partial(out_chunk, pit, pn, (u - 1) % 2, j) for j in range(T // 8)])
        run_unit(v_slot(it), n, u % 2, _interleave(side))
        if u > 0:
            o_copy(pit, pn).start()

    def item_body(it, par):
        nx = jnp.minimum(it + 1, NI - 1)
        nb = nx // NM
        nm = nx - nb * NM
        tasks = [(c, j) for c in range(NC) for j in range(T // 16)]
        for n in range(NC):
            mine = tasks[n * len(tasks) // V_UNITS:(n + 1) * len(tasks) // V_UNITS]
            side = [[functools.partial(v_chunk, nb, nm, (par + 1) % 2, c, j) for c, j in mine]] if mine else []
            pit, pn = (it, n - 1) if n > 0 else (it - 1, NC - 1)
            side.append([functools.partial(out_chunk, pit, pn, (n - 1) % 2, j) for j in range(T // 8)])
            run_unit(par, n, n % 2, _interleave(side))
            o_copy(pit, pn).start()

    def wait_x(nx):
        @pl.when(nx < NI)
        def _():
            nb = nx // NM
            nm = nx - nb * NM
            for m in range(NM):
                @pl.when(nm == m)
                def _():
                    for cp in x_copies(nb, m, nx):
                        cp.wait()

    @pl.loop(0, (NI - NA) // 2)
    def _(i):
        for k in range(2):
            wait_x(NA + 2 * i + k + 1)
        for k in range(2):
            item_body(NA + 2 * i + k, k)

    for j in range(T // 8):
        out_chunk(NI - 1, NC - 1, (NC - 1) % 2, j)
    o_copy(NI - 1, NC - 1).start()
    for it in range(NI):
        for n in range(NC):
            o_copy(it, n).wait()


@jax.jit
def pallas_standalone__batchnorm__prompt_kernel(
    x: jax.Array,
    w: jax.Array,
    mean: jax.Array,
    var: jax.Array,
    g: jax.Array,
    b: jax.Array,
):
    assert x.shape == (B, S, C) and w.shape == (3, C, C)
    return pl.pallas_call(
        _kernel,
        grid=(),
        in_specs=[pl.BlockSpec(memory_space=pl.ANY)] * 6,
        out_specs=pl.BlockSpec(memory_space=pl.ANY),
        out_shape=jax.ShapeDtypeStruct(x.shape, x.dtype),
        scratch_shapes=[
            pltpu.VMEM((B, NC, S + 2 * HALO, 128), BF16),
            pltpu.VMEM((3, NC, C, 128), BF16),
            pltpu.VMEM((4, NC, C // 2, 128), U32),
            pltpu.VMEM((4, 6, NC, T // 2, 128), U32),
            pltpu.VMEM((2, 6, T, 128), F32),
            pltpu.VMEM((NI, NC, 4 * T, 128), BF16),
            pltpu.VMEM((C,), BF16), pltpu.VMEM((C,), BF16),
            pltpu.VMEM((C,), BF16), pltpu.VMEM((C,), BF16),
            pltpu.SemaphoreType.DMA((NI,)),
            pltpu.SemaphoreType.DMA((NC,)),
            pltpu.SemaphoreType.DMA((1,)),
            pltpu.SemaphoreType.DMA((1,)),
        ],
        compiler_params=pltpu.CompilerParams(vmem_limit_bytes=100 * 1024 * 1024),
    )(x, w, mean, var, g, b)
```

```python
import functools

import jax
import jax.numpy as jnp
import jax.experimental.pallas as pl
import jax.experimental.pallas.tpu as pltpu

F32, BF16, U32 = jnp.float32, jnp.bfloat16, jnp.uint32

B, S, C = 2, 2048, 1024
NC = C // 128
T = 128
NM = S // 4 // T
NI = B * NM
NA = 2
HALO = 16

P, Q = 0.625, 1.5
P2, Q2 = P * P, Q * Q
F0, FP, FQ = P2 * Q2, 2 * P2 * (P2 - Q2), 2 * Q2 * (Q2 - P2)

UNITS_A = [(0, 0), (0, 1), (1, 0), (1, 1)] + [(it, n) for n in range(2, NC) for it in range(NA)]
WAITS = {1: ['W1'], 2: ['X1'], 3: ['W2'], 5: ['W3'], 7: ['W4', 'W5'], 11: ['W6', 'W7', 'X2']}
EARLY_U = []
PRE = {1: ['U1'], 2: ['V1']}
U_SIDE = {2 * n - 1: n for n in range(2, NC)}
V_SIDE = {11: [0, 1], 12: [2, 3, 4], 13: [5], 14: [6, 7]}
STARTS = {'pro': ['X0', 'W0', 'W1'], 'x0': ['X1'], 'w0': ['W2'], 0: ['W3'], 1: ['W4'], 2: ['W5'], 3: ['W6', 'W7'], 4: ['X2'], 7: ['X3'], 9: ['X4'], 11: ['X5'], 13: ['X6'], 15: ['X7']}
SLOT_OFFSET = 12
V_UNITS = 4


def _interleave(lists):
    tagged = []
    for tasks in lists:
        for j, t in enumerate(tasks):
            tagged.append(((j + 0.5) / len(tasks), t))
    tagged.sort(key=lambda a: a[0])
    return [t for _, t in tagged]


def _kernel(x_hbm, w_hbm, mean_hbm, var_hbm, g_hbm, b_hbm, o_hbm,
            xs, wr, us, vs, ms, os_, mean_v, var_v, g_v, b_v, xsem, wsem, osem, psem):
    xu, ou, wru = xs.bitcast(U32), os_.bitcast(U32), wr.bitcast(U32)
    as_bf16 = lambda v: pltpu.bitcast(v, BF16)
    lo = lambda u: pltpu.unpack_elementwise(u, index=0, packed_dtype=BF16, unpacked_dtype=F32)
    hi = lambda u: pltpu.unpack_elementwise(u, index=1, packed_dtype=BF16, unpacked_dtype=F32)
    pack = lambda a, b: pltpu.pack_elementwise([a, b], packed_dtype=BF16)

    def x_copies(b, m, it):
        r0 = 0 if m == 0 else m * 4 * T + HALO
        r1 = min((m + 1) * 4 * T + HALO, S)
        return [pltpu.make_async_copy(
            x_hbm.at[b, pl.ds(r0, r1 - r0), pl.ds(c * 128, 128)],
            xs.at[b, c, pl.ds(HALO + r0, r1 - r0), :], xsem.at[it]) for c in range(NC)]

    def w_copies(n):
        return [pltpu.make_async_copy(
            w_hbm.at[k, :, pl.ds(n * 128, 128)], wr.at[k, n], wsem.at[n]) for k in range(3)]

    def o_copy(it, n):
        b = it // NM
        m = it - b * NM
        return pltpu.make_async_copy(
            os_.at[it, n], o_hbm.at[b, pl.ds(m * 4 * T, 4 * T), pl.ds(n * 128, 128)], osem.at[0])

    def group(name):
        k = int(name[1:])
        return x_copies(k // NM, k % NM, k) if name[0] == 'X' else w_copies(k)

    def start(key):
        for name in STARTS.get(key, []):
            for cp in group(name):
                cp.start(priority=0 if name in ['X0'] else 1)

    def wait(name):
        for cp in group(name):
            cp.wait()

    start('pro')
    small = [pltpu.make_async_copy(src, dst, psem.at[0]) for src, dst in
             zip((mean_hbm, var_hbm, g_hbm, b_hbm), (mean_v, var_v, g_v, b_v))]
    for cp in small:
        cp.start()
    zero8 = jnp.zeros((8, 128), U32)
    for b in range(B):
        for c in range(NC):
            xu[b, c, pl.ds(0, 8), :] = zero8
            xu[b, c, pl.ds((HALO + S) // 2, 8), :] = zero8
    for cp in small:
        cp.wait()

    mean, var, g, beta = (r[...].astype(F32).reshape(1, C) for r in (mean_v, var_v, g_v, b_v))
    scale = g * (1.0 / jnp.sqrt(var + 1e-5))
    shift = beta - mean * scale
    scale, shift = 0.5 * scale, 0.5 * shift
    zero = jnp.where(pltpu.bitcast(jnp.broadcast_to(var[:, 0:128] * 0.0, (8, 128)), U32) == 12345,
                     jnp.uint32(1), jnp.uint32(0))

    def v_chunk(b, m, slot, c, j):
        if isinstance(m, int):
            xv = xu.at[b, c]
            base = HALO // 2 + m * 2 * T + j * 32
        else:
            xv = xu.at[b, c, pl.ds(pl.multiple_of(m * 2 * T, 8), 2 * T + HALO), :]
            base = HALO // 2 + j * 32
        res = []
        for par in range(2):
            o = base + 2 * par
            prev, cur, nxt, last = (xv[pl.ds(o + k, 8, stride=4), :] for k in (-1, 0, 1, 2))
            d0, d1, d2, d3, d4, d5 = hi(prev), lo(cur), hi(cur), lo(nxt), hi(nxt), lo(last)
            eq = d4 - Q2 * d2
            oq = d3 - Q2 * d1
            ep = d4 - P2 * d2
            op = d3 - P2 * d1
            v0 = ep - Q2 * (d2 - P2 * d0)
            v5 = (d5 - P2 * d3) - Q2 * op
            poq = P * oq
            qop = Q * op
            res.append((v0, eq + poq, eq - poq, ep + qop, ep - qop, v5))
        for i in range(6):
            r = pack(res[0][i], res[1][i])
            vs[slot, i, c, pl.ds(j * 8, 8), :] = r
        return r

    def u_chunk(n, j):
        w = [wru[k, n, pl.ds(j * 8, 8), :] for k in range(3)]
        res = []
        for half in (lo, hi):
            w0, w1, w2 = half(w[0]), half(w[1]), half(w[2])
            e, o = w0 + P2 * w2, P * w1
            e2, o2 = w0 + Q2 * w2, Q * w1
            res.append((e + o, e - o, e2 + o2, e2 - o2))
        for i in range(4):
            r = pack(res[0][i], res[1][i])
            us[i, n, pl.ds(j * 8, 8), :] = r
        return r

    def out_chunk(it, n, mslot, j):
        m0, m1, m2, m3, m4, m5 = (ms[mslot, i, pl.ds(j * 8, 8), :] for i in range(6))
        a = scale[:, n * 128:(n + 1) * 128]
        c0 = shift[:, n * 128:(n + 1) * 128]
        sp, tp = m1 + m2, m1 - m2
        sq, tq = m3 + m4, m3 - m4
        h0 = m0 * (a * (1 / F0)) + sp * (a * (1 / FP)) + sq * (a * (1 / FQ)) + c0
        h1 = tp * (a * (P / FP)) + tq * (a * (Q / FQ)) + c0
        h2 = sp * (a * (P2 / FP)) + sq * (a * (Q2 / FQ)) + c0
        h3 = tp * (a * (P2 * P / FP)) + tq * (a * (Q2 * Q / FQ)) + m5 * a + c0
        y0, y1, y2, y3 = (h + h * jnp.tanh(h) for h in (h0, h1, h2, h3))
        ov = ou.at[it, n]
        ov[pl.ds(16 * j, 8, stride=2), :] = pack(y0, y1)
        r = pack(y2, y3)
        ov[pl.ds(16 * j + 1, 8, stride=2), :] = r
        return r

    def weights(i, n):
        src = (wru.at[0], us.at[0], us.at[1], us.at[2], us.at[3], wru.at[2])[i]
        return as_bf16(src[n])

    def run_unit(slot, n, mslot, side, early=()):
        rc = T // 16
        nslots = 6 * 2 * rc
        tied = {}
        for j, t in enumerate(side):
            s = SLOT_OFFSET + int(j * (nslots - SLOT_OFFSET) / len(side))
            tied.setdefault(min(nslots - 1, s), []).append(t)
        for j, t in enumerate(early):
            tied.setdefault(int(j * 32 / len(early)), []).append(t)
        for pos, i in enumerate((0, 5, 1, 2, 3, 4) if early else range(6)):
            dep = {}
            for h in range(2):
                for r in range(rc):
                    for t in tied.get((pos * 2 + h) * rc + r, []):
                        d = t() & zero
                        key = (h * (NC // 2), r)
                        dep[key] = d if key not in dep else (dep[key] | d)
            parts = []
            for c in range(NC):
                full = vs[slot, i, c]
                if any(cc == c for cc, _ in dep):
                    full = jnp.concatenate(
                        [(full[8 * r:8 * r + 8] | dep[(c, r)]) if (c, r) in dep else full[8 * r:8 * r + 8]
                         for r in range(rc)], axis=0)
                parts.append(as_bf16(full))
            ms[mslot, i] = jnp.dot(jnp.concatenate(parts, axis=1), weights(i, n),
                                   preferred_element_type=F32)

    v_slot = lambda it: it + 2 if it < NA else it % 2

    def first_weights():
        wait('W0')
        start('w0')
        if 0 not in EARLY_U:
            for j in range(C // 16):
                u_chunk(0, j)
        start('u0')

    def first_rows():
        wait('X0')
        start('x0')
        for c in range(NC):
            for j in range(T // 16):
                v_chunk(0, 0, v_slot(0), c, j)
        start('v0')

    for step in 'XW':
        {'W': first_weights, 'X': first_rows}[step]()

    for u, (it, n) in enumerate(UNITS_A):
        for name in WAITS.get(u, []):
            wait(name)
        start(u)
        for name in PRE.get(u, []):
            k = int(name[1:])
            if name[0] == 'U':
                if u not in EARLY_U:
                    for j in range(C // 16):
                        u_chunk(k, j)
            else:
                for c in range(NC):
                    for j in range(T // 16):
                        v_chunk(k // NM, k % NM, v_slot(k), c, j)
        side = []
        if u in U_SIDE:
            side.append([functools.partial(u_chunk, U_SIDE[u], j) for j in range(C // 16)])
        if u in V_SIDE:
            side.append([functools.partial(v_chunk, NA // NM, NA % NM, v_slot(NA), c, j)
                         for c in V_SIDE[u] for j in range(T // 16)])
        if u > 0:
            pit, pn = UNITS_A[u - 1]
            side.append([functools.partial(out_chunk, pit, pn, (u - 1) % 2, j) for j in range(T // 8)])
        early = [functools.partial(u_chunk, n, j) for j in range(C // 16)] if u in EARLY_U else ()
        run_unit(v_slot(it), n, u % 2, _interleave(side), early)
        if u > 0:
            o_copy(pit, pn).start()

    def item_body(it, par):
        nx = jnp.minimum(it + 1, NI - 1)
        nb = nx // NM
        nm = nx - nb * NM
        tasks = [(c, j) for c in range(NC) for j in range(T // 16)]
        for n in range(NC):
            mine = tasks[n * len(tasks) // V_UNITS:(n + 1) * len(tasks) // V_UNITS]
            side = [[functools.partial(v_chunk, nb, nm, (par + 1) % 2, c, j) for c, j in mine]] if mine else []
            pit, pn = (it, n - 1) if n > 0 else (it - 1, NC - 1)
            side.append([functools.partial(out_chunk, pit, pn, (n - 1) % 2, j) for j in range(T // 8)])
            run_unit(par, n, n % 2, _interleave(side))
            o_copy(pit, pn).start()

    def wait_x(nx):
        @pl.when(nx < NI)
        def _():
            nb = nx // NM
            nm = nx - nb * NM
            for m in range(NM):
                @pl.when(nm == m)
                def _():
                    for cp in x_copies(nb, m, nx):
                        cp.wait()

    @pl.loop(0, (NI - NA) // 2)
    def _(i):
        for k in range(2):
            wait_x(NA + 2 * i + k + 1)
        for k in range(2):
            item_body(NA + 2 * i + k, k)

    for j in range(T // 8):
        out_chunk(NI - 1, NC - 1, (NC - 1) % 2, j)
    o_copy(NI - 1, NC - 1).start()
    for it in range(NI):
        for n in range(NC):
            o_copy(it, n).wait()


@jax.jit
def pallas_standalone__batchnorm__prompt_kernel(
    x: jax.Array,
    w: jax.Array,
    mean: jax.Array,
    var: jax.Array,
    g: jax.Array,
    b: jax.Array,
):
    assert x.shape == (B, S, C) and w.shape == (3, C, C)
    return pl.pallas_call(
        _kernel,
        grid=(),
        in_specs=[pl.BlockSpec(memory_space=pl.ANY)] * 6,
        out_specs=pl.BlockSpec(memory_space=pl.ANY),
        out_shape=jax.ShapeDtypeStruct(x.shape, x.dtype),
        scratch_shapes=[
            pltpu.VMEM((B, NC, S + 2 * HALO, 128), BF16),
            pltpu.VMEM((3, NC, C, 128), BF16),
            pltpu.VMEM((4, NC, C // 2, 128), U32),
            pltpu.VMEM((4, 6, NC, T // 2, 128), U32),
            pltpu.VMEM((2, 6, T, 128), F32),
            pltpu.VMEM((NI, NC, 4 * T, 128), BF16),
            pltpu.VMEM((C,), BF16), pltpu.VMEM((C,), BF16),
            pltpu.VMEM((C,), BF16), pltpu.VMEM((C,), BF16),
            pltpu.SemaphoreType.DMA((NI,)),
            pltpu.SemaphoreType.DMA((NC,)),
            pltpu.SemaphoreType.DMA((1,)),
            pltpu.SemaphoreType.DMA((1,)),
        ],
        compiler_params=pltpu.CompilerParams(vmem_limit_bytes=100 * 1024 * 1024),
    )(x, w, mean, var, g, b)
```

```python
import functools

import jax
import jax.numpy as jnp
import jax.experimental.pallas as pl
import jax.experimental.pallas.tpu as pltpu

F32, BF16, U32 = jnp.float32, jnp.bfloat16, jnp.uint32

B, S, C = 2, 2048, 1024
NC = C // 128
T = 128
NM = S // 4 // T
NI = B * NM
NA = 2
HALO = 16

P, Q = 0.625, 1.5
P2, Q2 = P * P, Q * Q
F0, FP, FQ = P2 * Q2, 2 * P2 * (P2 - Q2), 2 * Q2 * (Q2 - P2)

UNITS_A = [(0, 0), (0, 1), (1, 0), (1, 1)] + [(it, n) for n in range(2, NC) for it in range(NA)]
STARTS = {'pro': ['X0', 'W0', 'W1'], 'x0': ['X1'], 'w0': ['W2'], 0: ['W3'], 1: ['W4'], 2: ['W5'],
          3: ['W6', 'W7'], 4: ['X2'], 7: ['X3'], 9: ['X4'], 11: ['X5'], 13: ['X6'], 15: ['X7']}
WAITS = {1: ['W1'], 2: ['X1'], 3: ['W2'], 5: ['W3'], 7: ['W4', 'W5'], 11: ['W6', 'W7', 'X2']}
PRE = {1: ['U1'], 2: ['V1']}
U_SIDE = {2 * n - 1: n for n in range(2, NC)}
V_SIDE = {11: [0, 1], 12: [2, 3, 4], 13: [5], 14: [6, 7]}
SLOT_OFFSET = 12
V_UNITS = 4


def _interleave(lists):
    tagged = []
    for tasks in lists:
        for j, t in enumerate(tasks):
            tagged.append(((j + 0.5) / len(tasks), t))
    tagged.sort(key=lambda a: a[0])
    return [t for _, t in tagged]


def _kernel(x_hbm, w_hbm, mean_hbm, var_hbm, g_hbm, b_hbm, o_hbm,
            xs, wr, us, vs, ms, os_, mean_v, var_v, g_v, b_v, xsem, wsem, osem, psem):
    xu, ou, wru = xs.bitcast(U32), os_.bitcast(U32), wr.bitcast(U32)
    as_bf16 = lambda v: pltpu.bitcast(v, BF16)
    lo = lambda u: pltpu.unpack_elementwise(u, index=0, packed_dtype=BF16, unpacked_dtype=F32)
    hi = lambda u: pltpu.unpack_elementwise(u, index=1, packed_dtype=BF16, unpacked_dtype=F32)
    pack = lambda a, b: pltpu.pack_elementwise([a, b], packed_dtype=BF16)

    def x_copies(b, m, it):
        r0 = 0 if m == 0 else m * 4 * T + HALO
        r1 = min((m + 1) * 4 * T + HALO, S)
        return [pltpu.make_async_copy(
            x_hbm.at[b, pl.ds(r0, r1 - r0), pl.ds(c * 128, 128)],
            xs.at[b, c, pl.ds(HALO + r0, r1 - r0), :], xsem.at[it]) for c in range(NC)]

    def w_copies(n):
        return [pltpu.make_async_copy(
            w_hbm.at[k, :, pl.ds(n * 128, 128)], wr.at[k, n], wsem.at[n]) for k in range(3)]

    def o_copy(it, n):
        b = it // NM
        m = it - b * NM
        return pltpu.make_async_copy(
            os_.at[it, n], o_hbm.at[b, pl.ds(m * 4 * T, 4 * T), pl.ds(n * 128, 128)], osem.at[0])

    def group(name):
        k = int(name[1:])
        return x_copies(k // NM, k % NM, k) if name[0] == 'X' else w_copies(k)

    def start(key):
        for name in STARTS.get(key, []):
            for cp in group(name):
                cp.start(priority=0 if name == 'X0' else 1)

    def wait(name):
        for cp in group(name):
            cp.wait()

    start('pro')
    small = [pltpu.make_async_copy(src, dst, psem.at[0]) for src, dst in
             zip((mean_hbm, var_hbm, g_hbm, b_hbm), (mean_v, var_v, g_v, b_v))]
    for cp in small:
        cp.start()
    zero8 = jnp.zeros((8, 128), U32)
    for b in range(B):
        for c in range(NC):
            xu[b, c, pl.ds(0, 8), :] = zero8
            xu[b, c, pl.ds((HALO + S) // 2, 8), :] = zero8
    for cp in small:
        cp.wait()

    mean, var, g, beta = (r[...].astype(F32).reshape(1, C) for r in (mean_v, var_v, g_v, b_v))
    scale = g * (1.0 / jnp.sqrt(var + 1e-5))
    shift = beta - mean * scale
    scale, shift = 0.5 * scale, 0.5 * shift
    zero = jnp.where(pltpu.bitcast(jnp.broadcast_to(var[:, 0:128] * 0.0, (8, 128)), U32) == 12345,
                     jnp.uint32(1), jnp.uint32(0))

    def v_chunk(b, m, slot, c, j):
        if isinstance(m, int):
            xv = xu.at[b, c]
            base = HALO // 2 + m * 2 * T + j * 32
        else:
            xv = xu.at[b, c, pl.ds(pl.multiple_of(m * 2 * T, 8), 2 * T + HALO), :]
            base = HALO // 2 + j * 32
        res = []
        for par in range(2):
            o = base + 2 * par
            prev, cur, nxt, last = (xv[pl.ds(o + k, 8, stride=4), :] for k in (-1, 0, 1, 2))
            d0, d1, d2, d3, d4, d5 = hi(prev), lo(cur), hi(cur), lo(nxt), hi(nxt), lo(last)
            eq = d4 - Q2 * d2
            oq = d3 - Q2 * d1
            ep = d4 - P2 * d2
            op = d3 - P2 * d1
            v0 = ep - Q2 * (d2 - P2 * d0)
            v5 = (d5 - P2 * d3) - Q2 * op
            poq = P * oq
            qop = Q * op
            res.append((v0, eq + poq, eq - poq, ep + qop, ep - qop, v5))
        for i in range(6):
            r = pack(res[0][i], res[1][i])
            vs[slot, i, c, pl.ds(j * 8, 8), :] = r
        return r

    def u_chunk(n, j):
        w = [wru[k, n, pl.ds(j * 8, 8), :] for k in range(3)]
        res = []
        for half in (lo, hi):
            w0, w1, w2 = half(w[0]), half(w[1]), half(w[2])
            e, o = w0 + P2 * w2, P * w1
            e2, o2 = w0 + Q2 * w2, Q * w1
            res.append((e + o, e - o, e2 + o2, e2 - o2))
        for i in range(4):
            r = pack(res[0][i], res[1][i])
            us[i, n, pl.ds(j * 8, 8), :] = r
        return r

    def out_chunk(it, n, mslot, j):
        m0, m1, m2, m3, m4, m5 = (ms[mslot, i, pl.ds(j * 8, 8), :] for i in range(6))
        a = scale[:, n * 128:(n + 1) * 128]
        c0 = shift[:, n * 128:(n + 1) * 128]
        sp, tp = m1 + m2, m1 - m2
        sq, tq = m3 + m4, m3 - m4
        h0 = m0 * (a * (1 / F0)) + sp * (a * (1 / FP)) + sq * (a * (1 / FQ)) + c0
        h1 = tp * (a * (P / FP)) + tq * (a * (Q / FQ)) + c0
        h2 = sp * (a * (P2 / FP)) + sq * (a * (Q2 / FQ)) + c0
        h3 = tp * (a * (P2 * P / FP)) + tq * (a * (Q2 * Q / FQ)) + m5 * a + c0
        y0, y1, y2, y3 = (h + h * jnp.tanh(h) for h in (h0, h1, h2, h3))
        ov = ou.at[it, n]
        ov[pl.ds(16 * j, 8, stride=2), :] = pack(y0, y1)
        r = pack(y2, y3)
        ov[pl.ds(16 * j + 1, 8, stride=2), :] = r
        return r

    def weights(i, n):
        src = (wru.at[0], us.at[0], us.at[1], us.at[2], us.at[3], wru.at[2])[i]
        return as_bf16(src[n])

    def run_unit(slot, n, mslot, side):
        rc = T // 16
        nslots = 6 * 2 * rc
        tied = {}
        for j, t in enumerate(side):
            s = SLOT_OFFSET + int(j * (nslots - SLOT_OFFSET) / len(side))
            tied.setdefault(min(nslots - 1, s), []).append(t)
        for i in range(6):
            dep = {}
            for h in range(2):
                for r in range(rc):
                    for t in tied.get((i * 2 + h) * rc + r, []):
                        d = t() & zero
                        key = (h * (NC // 2), r)
                        dep[key] = d if key not in dep else (dep[key] | d)
            parts = []
            for c in range(NC):
                full = vs[slot, i, c]
                if any(cc == c for cc, _ in dep):
                    full = jnp.concatenate(
                        [(full[8 * r:8 * r + 8] | dep[(c, r)]) if (c, r) in dep else full[8 * r:8 * r + 8]
                         for r in range(rc)], axis=0)
                parts.append(as_bf16(full))
            ms[mslot, i] = jnp.dot(jnp.concatenate(parts, axis=1), weights(i, n),
                                   preferred_element_type=F32)

    v_slot = lambda it: it + 2 if it < NA else it % 2

    wait('X0')
    start('x0')
    for c in range(NC):
        for j in range(T // 16):
            v_chunk(0, 0, v_slot(0), c, j)
    wait('W0')
    start('w0')
    for j in range(C // 16):
        u_chunk(0, j)

    for u, (it, n) in enumerate(UNITS_A):
        for name in WAITS.get(u, []):
            wait(name)
        start(u)
        for name in PRE.get(u, []):
            k = int(name[1:])
            if name[0] == 'U':
                for j in range(C // 16):
                    u_chunk(k, j)
            else:
                for c in range(NC):
                    for j in range(T // 16):
                        v_chunk(k // NM, k % NM, v_slot(k), c, j)
        side = []
        if u in U_SIDE:
            side.append([functools.partial(u_chunk, U_SIDE[u], j) for j in range(C // 16)])
        if u in V_SIDE:
            side.append([functools.partial(v_chunk, NA // NM, NA % NM, v_slot(NA), c, j)
                         for c in V_SIDE[u] for j in range(T // 16)])
        if u > 0:
            pit, pn = UNITS_A[u - 1]
            side.append([functools.partial(out_chunk, pit, pn, (u - 1) % 2, j) for j in range(T // 8)])
        run_unit(v_slot(it), n, u % 2, _interleave(side))
        if u > 0:
            o_copy(pit, pn).start()

    def item_body(it, par):
        nx = jnp.minimum(it + 1, NI - 1)
        nb = nx // NM
        nm = nx - nb * NM
        tasks = [(c, j) for c in range(NC) for j in range(T // 16)]
        for n in range(NC):
            mine = tasks[n * len(tasks) // V_UNITS:(n + 1) * len(tasks) // V_UNITS]
            side = [[functools.partial(v_chunk, nb, nm, (par + 1) % 2, c, j) for c, j in mine]] if mine else []
            pit, pn = (it, n - 1) if n > 0 else (it - 1, NC - 1)
            side.append([functools.partial(out_chunk, pit, pn, (n - 1) % 2, j) for j in range(T // 8)])
            run_unit(par, n, n % 2, _interleave(side))
            o_copy(pit, pn).start()

    def wait_x(nx):
        @pl.when(nx < NI)
        def _():
            nb = nx // NM
            nm = nx - nb * NM
            for m in range(NM):
                @pl.when(nm == m)
                def _():
                    for cp in x_copies(nb, m, nx):
                        cp.wait()

    @pl.loop(0, (NI - NA) // 2)
    def _(i):
        for k in range(2):
            wait_x(NA + 2 * i + k + 1)
        for k in range(2):
            item_body(NA + 2 * i + k, k)

    for j in range(T // 8):
        out_chunk(NI - 1, NC - 1, (NC - 1) % 2, j)
    o_copy(NI - 1, NC - 1).start()
    for it in range(NI):
        for n in range(NC):
            o_copy(it, n).wait()


@jax.jit
def pallas_standalone__batchnorm__prompt_kernel(
    x: jax.Array,
    w: jax.Array,
    mean: jax.Array,
    var: jax.Array,
    g: jax.Array,
    b: jax.Array,
):
    assert x.shape == (B, S, C) and w.shape == (3, C, C)
    return pl.pallas_call(
        _kernel,
        grid=(),
        in_specs=[pl.BlockSpec(memory_space=pl.ANY)] * 6,
        out_specs=pl.BlockSpec(memory_space=pl.ANY),
        out_shape=jax.ShapeDtypeStruct(x.shape, x.dtype),
        scratch_shapes=[
            pltpu.VMEM((B, NC, S + 2 * HALO, 128), BF16),
            pltpu.VMEM((3, NC, C, 128), BF16),
            pltpu.VMEM((4, NC, C // 2, 128), U32),
            pltpu.VMEM((4, 6, NC, T // 2, 128), U32),
            pltpu.VMEM((2, 6, T, 128), F32),
            pltpu.VMEM((NI, NC, 4 * T, 128), BF16),
            pltpu.VMEM((C,), BF16), pltpu.VMEM((C,), BF16),
            pltpu.VMEM((C,), BF16), pltpu.VMEM((C,), BF16),
            pltpu.SemaphoreType.DMA((NI,)),
            pltpu.SemaphoreType.DMA((NC,)),
            pltpu.SemaphoreType.DMA((1,)),
            pltpu.SemaphoreType.DMA((1,)),
        ],
        compiler_params=pltpu.CompilerParams(vmem_limit_bytes=100 * 1024 * 1024),
    )(x, w, mean, var, g, b)
```
